```python
import os as _os
_os.environ.setdefault("JAX_PLATFORMS", "cpu")
import jax
import jax.numpy as jnp

def _softmax(x, axis=-1):
    return jax.nn.softmax(x, axis=axis)
def _gelu(x):
    return jax.nn.gelu(x, approximate=True)
def _silu(x):
    return jax.nn.silu(x)
def _sigmoid(x):
    return jax.nn.sigmoid(x)
def _layernorm(x, axis=-1, eps=1e-5):
    m = jnp.mean(x, axis=axis, keepdims=True)
    v = jnp.var(x, axis=axis, keepdims=True)
    return (x - m) / jnp.sqrt(v + eps)
def _scatter_add(tgt, idx, src, axis=0):
    return tgt.at[idx].add(src)
def _segment_sum(src, seg, n):
    return jax.ops.segment_sum(src, seg, n)
class _Rng:
    def __init__(self, key):
        self._k = key
    def _next(self):
        self._k, sub = jax.random.split(self._k)
        return sub
    def normal(self, shape):
        return jax.random.normal(self._next(), shape, dtype=jnp.bfloat16)
    def randint(self, lo, hi, shape):
        return jax.random.randint(self._next(), shape, lo, hi, dtype=jnp.int32)
    def uniform(self, shape, lo=0.0, hi=1.0):
        return jax.random.uniform(self._next(), shape, jnp.bfloat16, lo, hi)
    def permutation(self, n):
        return jax.random.permutation(self._next(), n)


kernel_name = 'standalone__gqa_softmax__near_ridge'

def setup_inputs():
    _rng = _Rng(jax.random.key(int.from_bytes(__import__("os").urandom(4), "little")))
    _w = (lambda a: (lambda t: t.astype(jnp.bfloat16) if jnp.issubdtype(t.dtype, jnp.floating) else t)(jnp.asarray(a)))
    B, Hq, Hkv, Sq, Sk, D = 8, 16, 8, 160, 2048, 256
    return {
        "q": _w((lambda *s: _rng.normal(s) * 0.05)(B, Hq, Sq, D)),
        "k": _w((lambda *s: _rng.normal(s) * 3.2)(B, Hkv, Sk, D)),
        "v": _w((lambda *s: _rng.normal(s) * 0.05)(B, Hkv, Sk, D)),
    }

def reference(q, k, v):
    B, Hq, Sq, D = q.shape
    Hkv = k.shape[1]
    rep = Hq // Hkv
    k = jnp.repeat(k, rep, axis=1)
    v = jnp.repeat(v, rep, axis=1)
    scale = D ** -0.5
    scores = jnp.einsum("bhqd,bhkd->bhqk", q, k) * scale
    p = _softmax(scores, axis=-1)
    return jnp.einsum("bhqk,bhkd->bhqd", p, v)
```

```python
import jax
import jax.numpy as jnp
import jax.experimental.pallas as pl
import jax.experimental.pallas.tpu as pltpu


def _attn_kernel(q_ref, k_ref, v_ref, o_ref):
    rep, sq, d = q_ref.shape
    q = q_ref[...].reshape(rep * sq, d) * jnp.bfloat16(d ** -0.5)
    s = jax.lax.dot_general(
        q, k_ref[...], (((1,), (1,)), ((), ())),
        preferred_element_type=jnp.float32)
    m = jnp.max(s, axis=-1, keepdims=True)
    p = jnp.exp(s - m)
    l = jnp.sum(p, axis=-1, keepdims=True)
    o = jnp.dot(p.astype(jnp.bfloat16), v_ref[...],
                preferred_element_type=jnp.float32)
    o = o / l
    o_ref[...] = o.reshape(rep, sq, d).astype(o_ref.dtype)


@jax.jit
def pallas_standalone__gqa_softmax__near_ridge_kernel(
    q: jax.Array,
    k: jax.Array,
    v: jax.Array,
):
    B, Hq, Sq, D = q.shape
    Hkv, Sk = k.shape[1], k.shape[2]
    rep = Hq // Hkv
    return pl.pallas_call(
        _attn_kernel,
        grid=(B, Hkv),
        in_specs=[
            pl.BlockSpec((None, rep, Sq, D), lambda b, h: (b, h, 0, 0)),
            pl.BlockSpec((None, None, Sk, D), lambda b, h: (b, h, 0, 0)),
            pl.BlockSpec((None, None, Sk, D), lambda b, h: (b, h, 0, 0)),
        ],
        out_specs=pl.BlockSpec((None, rep, Sq, D), lambda b, h: (b, h, 0, 0)),
        out_shape=jax.ShapeDtypeStruct(q.shape, q.dtype),
        compiler_params=pltpu.CompilerParams(
            dimension_semantics=("parallel", "parallel"),
            vmem_limit_bytes=64 * 1024 * 1024),
    )(q, k, v)
```

```python
import functools
import math

import jax
import jax.numpy as jnp
import jax.experimental.pallas as pl
import jax.experimental.pallas.tpu as pltpu

_LOG2E = math.log2(math.e)


def _qk(q, k):
    return jax.lax.dot_general(
        q, k, (((1,), (1,)), ((), ())), preferred_element_type=jnp.float32)


def _lane_fold(x, op):
    r = x[:, 0:128]
    for t in range(1, x.shape[1] // 128):
        r = op(r, x[:, t * 128:(t + 1) * 128])
    return r


def _attn_kernel(q_ref, k_ref, v_ref, o_ref, *, hb, C):
    _, M, d = q_ref.shape
    Sk = k_ref.shape[1]
    c = (d ** -0.5) * _LOG2E
    n = Sk // C
    items = [(t, j) for t in range(hb) for j in range(n)]
    svals = {}

    def do_qk(idx):
        t, j = items[idx]
        svals[idx] = _qk(q_ref[t], k_ref[t, j * C:(j + 1) * C, :])

    do_qk(0)
    m = l = acc = None
    for idx, (t, j) in enumerate(items):
        if idx + 1 < len(items):
            do_qk(idx + 1)
        s = svals.pop(idx)
        mj = jnp.max(_lane_fold(s, jnp.maximum), axis=-1, keepdims=True)
        m_new = mj if j == 0 else jnp.maximum(m, mj)
        p = jnp.exp2((s - m_new) * c)
        lj = _lane_fold(p, jnp.add)
        oj = jnp.dot(p.astype(jnp.bfloat16), v_ref[t, j * C:(j + 1) * C, :],
                     preferred_element_type=jnp.float32)
        if j == 0:
            l = lj
            acc = oj
        else:
            alpha = jnp.exp2((m - m_new) * c)
            l = l * alpha + lj
            acc = acc * alpha + oj
        m = m_new
        if j == n - 1:
            lf = jnp.sum(l, axis=-1, keepdims=True)
            o_ref[t] = (acc / lf).astype(o_ref.dtype)


@jax.jit
def pallas_standalone__gqa_softmax__near_ridge_kernel(
    q: jax.Array,
    k: jax.Array,
    v: jax.Array,
):
    B, Hq, Sq, D = q.shape
    Hkv, Sk = k.shape[1], k.shape[2]
    rep = Hq // Hkv
    N = B * Hkv
    M = rep * Sq
    hb, C = 2, 256
    q3 = q.reshape(N, M, D)
    k3 = k.reshape(N, Sk, D)
    v3 = v.reshape(N, Sk, D)
    out = pl.pallas_call(
        functools.partial(_attn_kernel, hb=hb, C=C),
        grid=(N // hb,),
        in_specs=[
            pl.BlockSpec((hb, M, D), lambda i: (i, 0, 0)),
            pl.BlockSpec((hb, Sk, D), lambda i: (i, 0, 0)),
            pl.BlockSpec((hb, Sk, D), lambda i: (i, 0, 0)),
        ],
        out_specs=pl.BlockSpec((hb, M, D), lambda i: (i, 0, 0)),
        out_shape=jax.ShapeDtypeStruct((N, M, D), q.dtype),
        compiler_params=pltpu.CompilerParams(
            dimension_semantics=("arbitrary",),
            vmem_limit_bytes=64 * 1024 * 1024),
    )(q3, k3, v3)
    return out.reshape(B, Hq, Sq, D)
```

```python
import functools
import math

import jax
import jax.numpy as jnp
import jax.experimental.pallas as pl
import jax.experimental.pallas.tpu as pltpu

_LOG2E = math.log2(math.e)
_NG = 4


def _qk(q, k):
    return jax.lax.dot_general(
        q, k, (((1,), (1,)), ((), ())), preferred_element_type=jnp.float32)


def _lane_fold(x, op):
    r = x[:, 0:128]
    for t in range(1, x.shape[1] // 128):
        r = op(r, x[:, t * 128:(t + 1) * 128])
    return r


def _attn_kernel(q_hbm, k_hbm, v_hbm, o_hbm, sb, ob, s0_scr,
                 sem_in, sem_pre, sem_out, *, C, startpos):
    N, M, d = q_hbm.shape
    Sk = k_hbm.shape[1]
    c = (d ** -0.5) * _LOG2E
    n = Sk // C
    o_k1 = 0
    o_v = Sk - C
    o_q = o_v + Sk
    o_k0 = o_q + M

    def slot_of(g):
        if isinstance(g, int):
            return g % _NG
        return jnp.bitwise_and(g, _NG - 1)

    def set_copies(g):
        s = slot_of(g)
        if isinstance(g, int):
            h1 = min(g + 1, N - 1)
        else:
            h1 = jnp.minimum(g + 1, N - 1)
        return [
            pltpu.make_async_copy(k_hbm.at[g, C:Sk], sb.at[s, o_k1:o_k1 + Sk - C], sem_in.at[s]),
            pltpu.make_async_copy(v_hbm.at[g], sb.at[s, o_v:o_v + Sk], sem_in.at[s]),
            pltpu.make_async_copy(q_hbm.at[h1], sb.at[s, o_q:o_q + M], sem_in.at[s]),
            pltpu.make_async_copy(k_hbm.at[h1, 0:C], sb.at[s, o_k0:o_k0 + C], sem_in.at[s]),
        ]

    ps = _NG - 1
    c0 = pltpu.make_async_copy(q_hbm.at[0], sb.at[ps, o_q:o_q + M], sem_pre.at[0])
    c1 = pltpu.make_async_copy(k_hbm.at[0, 0:C], sb.at[ps, o_k0:o_k0 + C], sem_pre.at[1])
    c0.start()
    c1.start()
    for cp in set_copies(0):
        cp.start()
    c0.wait()
    c1.wait()
    s0_scr[...] = _qk(sb[ps, o_q:o_q + M, :], sb[ps, o_k0:o_k0 + C, :])

    def body(g, carry):
        s = slot_of(g)
        sq = slot_of(g + (_NG - 1))
        pltpu.make_async_copy(sb.at[s], sb.at[s], sem_in.at[s]).wait()
        q = sb[sq, o_q:o_q + M, :]

        svals = {0: s0_scr[...]}
        m = l = acc = None
        for j in range(n):
            if j == startpos:
                @pl.when(g + 2 < N)
                def _():
                    for cp in set_copies(g + 2):
                        cp.start()
            if j + 1 < n:
                svals[j + 1] = _qk(q, sb[s, o_k1 + j * C:o_k1 + (j + 1) * C, :])
            if j == 0:
                @pl.when(g == 0)
                def _():
                    for cp in set_copies(1):
                        cp.start()
            sv = svals.pop(j)
            mj = jnp.max(_lane_fold(sv, jnp.maximum), axis=-1, keepdims=True)
            m_new = mj if j == 0 else jnp.maximum(m, mj)
            p = jnp.exp2((sv - m_new) * c)
            lj = _lane_fold(p, jnp.add)
            oj = jnp.dot(p.astype(jnp.bfloat16), sb[s, o_v + j * C:o_v + (j + 1) * C, :],
                         preferred_element_type=jnp.float32)
            if j == 0:
                l = lj
                acc = oj
            else:
                alpha = jnp.exp2((m - m_new) * c)
                l = l * alpha + lj
                acc = acc * alpha + oj
            m = m_new
        s0_scr[...] = _qk(sb[s, o_q:o_q + M, :], sb[s, o_k0:o_k0 + C, :])
        lf = jnp.sum(l, axis=-1, keepdims=True)
        ob[g] = (acc / lf).astype(ob.dtype)
        pltpu.make_async_copy(ob.at[g], o_hbm.at[g], sem_out).start()
        return carry

    jax.lax.fori_loop(0, N, body, 0)
    pltpu.make_async_copy(ob, o_hbm, sem_out).wait()


@jax.jit
def pallas_standalone__gqa_softmax__near_ridge_kernel(
    q: jax.Array,
    k: jax.Array,
    v: jax.Array,
):
    B, Hq, Sq, D = q.shape
    Hkv, Sk = k.shape[1], k.shape[2]
    rep = Hq // Hkv
    N = B * Hkv
    M = rep * Sq
    C = 256
    q3 = q.reshape(N, M, D)
    k3 = k.reshape(N, Sk, D)
    v3 = v.reshape(N, Sk, D)
    out = pl.pallas_call(
        functools.partial(_attn_kernel, C=C, startpos=6),
        in_specs=[pl.BlockSpec(memory_space=pl.ANY)] * 3,
        out_specs=pl.BlockSpec(memory_space=pl.ANY),
        out_shape=jax.ShapeDtypeStruct((N, M, D), q.dtype),
        scratch_shapes=[
            pltpu.VMEM((_NG, 2 * Sk + M, D), q.dtype),
            pltpu.VMEM((N, M, D), q.dtype),
            pltpu.VMEM((M, C), jnp.float32),
            pltpu.SemaphoreType.DMA((_NG,)),
            pltpu.SemaphoreType.DMA((2,)),
            pltpu.SemaphoreType.DMA(()),
        ],
        compiler_params=pltpu.CompilerParams(
            vmem_limit_bytes=64 * 1024 * 1024,
            disable_bounds_checks=True),
    )(q3, k3, v3)
    return out.reshape(B, Hq, Sq, D)
```

```python
import functools
import math

import jax
import jax.numpy as jnp
import jax.experimental.pallas as pl
import jax.experimental.pallas.tpu as pltpu

_LOG2E = math.log2(math.e)
_NG = 4


def _qk(q, k):
    return jax.lax.dot_general(
        q, k, (((1,), (1,)), ((), ())), preferred_element_type=jnp.float32)


def _lane_fold(x, op):
    r = x[:, 0:128]
    for t in range(1, x.shape[1] // 128):
        r = op(r, x[:, t * 128:(t + 1) * 128])
    return r


def _attn_kernel(q_hbm, k_hbm, v_hbm, o_hbm, sb, ob, s0_scr,
                 sem_in, sem_a, sem_b, sem_pre, sem_out, *, C, startpos, kf):
    N, M, d = q_hbm.shape
    Sk = k_hbm.shape[1]
    c = (d ** -0.5) * _LOG2E
    n = Sk // C
    H = n // 2
    o_k1 = 0
    o_v = Sk - C
    o_q = o_v + Sk
    o_k0 = o_q + M

    def slot_of(g):
        if isinstance(g, int):
            return g % _NG
        return jnp.bitwise_and(g, _NG - 1)

    def nxt(g):
        if isinstance(g, int):
            return min(g + 1, N - 1)
        return jnp.minimum(g + 1, N - 1)

    def set_copies(g):
        s = slot_of(g)
        h1 = nxt(g)
        return [
            pltpu.make_async_copy(k_hbm.at[g, C:Sk], sb.at[s, o_k1:o_k1 + Sk - C], sem_in.at[s]),
            pltpu.make_async_copy(v_hbm.at[g], sb.at[s, o_v:o_v + Sk], sem_in.at[s]),
            pltpu.make_async_copy(q_hbm.at[h1], sb.at[s, o_q:o_q + M], sem_in.at[s]),
            pltpu.make_async_copy(k_hbm.at[h1, 0:C], sb.at[s, o_k0:o_k0 + C], sem_in.at[s]),
        ]

    def a_copies(g):
        s = slot_of(g)
        return [
            pltpu.make_async_copy(k_hbm.at[g, C:(H + 1) * C], sb.at[s, o_k1:o_k1 + H * C], sem_a.at[s]),
            pltpu.make_async_copy(v_hbm.at[g, 0:H * C], sb.at[s, o_v:o_v + H * C], sem_a.at[s]),
        ]

    def b_copies(g):
        s = slot_of(g)
        h1 = nxt(g)
        return [
            pltpu.make_async_copy(k_hbm.at[g, (H + 1) * C:Sk], sb.at[s, o_k1 + H * C:o_k1 + Sk - C], sem_b.at[s]),
            pltpu.make_async_copy(v_hbm.at[g, H * C:Sk], sb.at[s, o_v + H * C:o_v + Sk], sem_b.at[s]),
            pltpu.make_async_copy(q_hbm.at[h1], sb.at[s, o_q:o_q + M], sem_b.at[s]),
            pltpu.make_async_copy(k_hbm.at[h1, 0:C], sb.at[s, o_k0:o_k0 + C], sem_b.at[s]),
        ]

    ps = _NG - 1
    c0 = pltpu.make_async_copy(q_hbm.at[0], sb.at[ps, o_q:o_q + M], sem_pre.at[0])
    c1 = pltpu.make_async_copy(k_hbm.at[0, 0:C], sb.at[ps, o_k0:o_k0 + C], sem_pre.at[1])
    c0.start()
    c1.start()
    for cp in a_copies(0):
        cp.start()
    c0.wait()
    c1.wait()
    for cp in b_copies(0):
        cp.start()
    s0_scr[...] = _qk(sb[ps, o_q:o_q + M, :], sb[ps, o_k0:o_k0 + C, :])

    def body(g, carry, *, fine):
        s = slot_of(g)
        sq = slot_of(g + (_NG - 1))
        if fine:
            for cp in a_copies(g):
                cp.wait()
        else:
            pltpu.make_async_copy(sb.at[s], sb.at[s], sem_in.at[s]).wait()
        q = sb[sq, o_q:o_q + M, :]

        def dma_hooks(j):
            if fine:
                if j == 1:
                    @pl.when(g + 1 < kf)
                    def _():
                        for cp in a_copies(g + 1):
                            cp.start()
                if j == H:
                    for cp in b_copies(g):
                        cp.wait()
                if j == H + 1:
                    @pl.when(g + 1 < kf)
                    def _():
                        for cp in b_copies(g + 1):
                            cp.start()
                if j == startpos:
                    @pl.when(g + 2 >= kf)
                    def _():
                        for cp in set_copies(g + 2):
                            cp.start()
            elif j == startpos:
                @pl.when(g + 2 < N)
                def _():
                    for cp in set_copies(g + 2):
                        cp.start()

        svals = {0: s0_scr[...]}
        m = l = acc = None
        for j in range(n):
            dma_hooks(j)
            if j + 1 < n:
                svals[j + 1] = _qk(q, sb[s, o_k1 + j * C:o_k1 + (j + 1) * C, :])
            sv = svals.pop(j)
            mj = jnp.max(_lane_fold(sv, jnp.maximum), axis=-1, keepdims=True)
            m_new = mj if j == 0 else jnp.maximum(m, mj)
            p = jnp.exp2((sv - m_new) * c)
            lj = _lane_fold(p, jnp.add)
            oj = jnp.dot(p.astype(jnp.bfloat16), sb[s, o_v + j * C:o_v + (j + 1) * C, :],
                         preferred_element_type=jnp.float32)
            if j == 0:
                l = lj
                acc = oj
            else:
                alpha = jnp.exp2((m - m_new) * c)
                l = l * alpha + lj
                acc = acc * alpha + oj
            m = m_new
        s0_scr[...] = _qk(sb[s, o_q:o_q + M, :], sb[s, o_k0:o_k0 + C, :])
        lf = jnp.sum(l, axis=-1, keepdims=True)
        ob[g] = (acc / lf).astype(ob.dtype)
        pltpu.make_async_copy(ob.at[g], o_hbm.at[g], sem_out).start()
        return carry

    jax.lax.fori_loop(0, kf, functools.partial(body, fine=True), 0)
    jax.lax.fori_loop(kf, N, functools.partial(body, fine=False), 0)
    pltpu.make_async_copy(ob, o_hbm, sem_out).wait()


@jax.jit
def pallas_standalone__gqa_softmax__near_ridge_kernel(
    q: jax.Array,
    k: jax.Array,
    v: jax.Array,
):
    B, Hq, Sq, D = q.shape
    Hkv, Sk = k.shape[1], k.shape[2]
    rep = Hq // Hkv
    N = B * Hkv
    M = rep * Sq
    C = 256
    q3 = q.reshape(N, M, D)
    k3 = k.reshape(N, Sk, D)
    v3 = v.reshape(N, Sk, D)
    out = pl.pallas_call(
        functools.partial(_attn_kernel, C=C, startpos=6, kf=4),
        in_specs=[pl.BlockSpec(memory_space=pl.ANY)] * 3,
        out_specs=pl.BlockSpec(memory_space=pl.ANY),
        out_shape=jax.ShapeDtypeStruct((N, M, D), q.dtype),
        scratch_shapes=[
            pltpu.VMEM((_NG, 2 * Sk + M, D), q.dtype),
            pltpu.VMEM((N, M, D), q.dtype),
            pltpu.VMEM((M, C), jnp.float32),
            pltpu.SemaphoreType.DMA((_NG,)),
            pltpu.SemaphoreType.DMA((_NG,)),
            pltpu.SemaphoreType.DMA((_NG,)),
            pltpu.SemaphoreType.DMA((2,)),
            pltpu.SemaphoreType.DMA(()),
        ],
        compiler_params=pltpu.CompilerParams(
            vmem_limit_bytes=64 * 1024 * 1024,
            disable_bounds_checks=True),
    )(q3, k3, v3)
    return out.reshape(B, Hq, Sq, D)
```

```python
import functools
import math

import jax
import jax.numpy as jnp
import jax.experimental.pallas as pl
import jax.experimental.pallas.tpu as pltpu

_LOG2E = math.log2(math.e)
_NG = 4


def _qk(q, k):
    return jax.lax.dot_general(
        q, k, (((1,), (1,)), ((), ())), preferred_element_type=jnp.float32)


def _lane_fold(x, op):
    r = x[:, 0:128]
    for t in range(1, x.shape[1] // 128):
        r = op(r, x[:, t * 128:(t + 1) * 128])
    return r


def _attn_kernel(q_hbm, k_hbm, v_hbm, o_hbm, sb, ob, s0_scr, kt_scr,
                 sem_in, sem_a, sem_b, sem_pre, sem_out,
                 *, C, startpos, tpos, kf):
    N, M, d = q_hbm.shape
    Sk = k_hbm.shape[1]
    c = (d ** -0.5) * _LOG2E
    n = Sk // C
    H = n // 2
    T = 2 * C
    o_k1 = 0
    o_v = Sk - T
    o_q = o_v + Sk
    o_k0 = o_q + M

    def slot_of(g):
        if isinstance(g, int):
            return g % _NG
        return jnp.bitwise_and(g, _NG - 1)

    def nxt(g):
        if isinstance(g, int):
            return min(g + 1, N - 1)
        return jnp.minimum(g + 1, N - 1)

    def set_copies(g):
        s = slot_of(g)
        h1 = nxt(g)
        return [
            pltpu.make_async_copy(k_hbm.at[g, T:Sk], sb.at[s, o_k1:o_k1 + Sk - T], sem_in.at[s]),
            pltpu.make_async_copy(v_hbm.at[g], sb.at[s, o_v:o_v + Sk], sem_in.at[s]),
            pltpu.make_async_copy(q_hbm.at[h1], sb.at[s, o_q:o_q + M], sem_in.at[s]),
            pltpu.make_async_copy(k_hbm.at[h1, 0:T], sb.at[s, o_k0:o_k0 + T], sem_in.at[s]),
        ]

    def a_copies(g):
        s = slot_of(g)
        return [
            pltpu.make_async_copy(k_hbm.at[g, T:(H + 1) * C],
                                  sb.at[s, o_k1:o_k1 + (H + 1) * C - T], sem_a.at[s]),
            pltpu.make_async_copy(v_hbm.at[g, 0:H * C], sb.at[s, o_v:o_v + H * C], sem_a.at[s]),
        ]

    def b_copies(g):
        s = slot_of(g)
        h1 = nxt(g)
        return [
            pltpu.make_async_copy(k_hbm.at[g, (H + 1) * C:Sk],
                                  sb.at[s, o_k1 + (H + 1) * C - T:o_k1 + Sk - T], sem_b.at[s]),
            pltpu.make_async_copy(v_hbm.at[g, H * C:Sk], sb.at[s, o_v + H * C:o_v + Sk], sem_b.at[s]),
            pltpu.make_async_copy(q_hbm.at[h1], sb.at[s, o_q:o_q + M], sem_b.at[s]),
            pltpu.make_async_copy(k_hbm.at[h1, 0:T], sb.at[s, o_k0:o_k0 + T], sem_b.at[s]),
        ]

    def transpose_into(slot):
        kt_scr[...] = sb[slot, o_k0 + C:o_k0 + T, :].astype(jnp.float32).T.astype(kt_scr.dtype)

    ps = _NG - 1
    c0 = pltpu.make_async_copy(q_hbm.at[0], sb.at[ps, o_q:o_q + M], sem_pre.at[0])
    c1 = pltpu.make_async_copy(k_hbm.at[0, 0:T], sb.at[ps, o_k0:o_k0 + T], sem_pre.at[1])
    c0.start()
    c1.start()
    for cp in a_copies(0):
        cp.start()
    c0.wait()
    c1.wait()
    for cp in b_copies(0):
        cp.start()
    s0_scr[...] = _qk(sb[ps, o_q:o_q + M, :], sb[ps, o_k0:o_k0 + C, :])
    transpose_into(ps)

    def body(g, carry, *, fine):
        s = slot_of(g)
        sq = slot_of(g + (_NG - 1))
        if fine:
            for cp in a_copies(g):
                cp.wait()
        else:
            pltpu.make_async_copy(sb.at[s], sb.at[s], sem_in.at[s]).wait()
        q = sb[sq, o_q:o_q + M, :]

        def dma_hooks(j):
            if fine:
                if j == 1:
                    @pl.when(g + 1 < kf)
                    def _():
                        for cp in a_copies(g + 1):
                            cp.start()
                if j == H:
                    for cp in b_copies(g):
                        cp.wait()
                if j == H + 1:
                    @pl.when(g + 1 < kf)
                    def _():
                        for cp in b_copies(g + 1):
                            cp.start()
                if j == startpos:
                    @pl.when(g + 2 >= kf)
                    def _():
                        for cp in set_copies(g + 2):
                            cp.start()
            elif j == startpos:
                @pl.when(g + 2 < N)
                def _():
                    for cp in set_copies(g + 2):
                        cp.start()

        svals = {0: s0_scr[...]}
        m = l = acc = None
        for j in range(n):
            dma_hooks(j)
            if j == 0:
                svals[1] = jnp.dot(q, kt_scr[...], preferred_element_type=jnp.float32)
            elif j + 1 < n:
                svals[j + 1] = _qk(q, sb[s, o_k1 + (j - 1) * C:o_k1 + j * C, :])
            if j == tpos:
                transpose_into(s)
            sv = svals.pop(j)
            mj = jnp.max(_lane_fold(sv, jnp.maximum), axis=-1, keepdims=True)
            m_new = mj if j == 0 else jnp.maximum(m, mj)
            p = jnp.exp2((sv - m_new) * c)
            lj = _lane_fold(p, jnp.add)
            oj = jnp.dot(p.astype(jnp.bfloat16), sb[s, o_v + j * C:o_v + (j + 1) * C, :],
                         preferred_element_type=jnp.float32)
            if j == 0:
                l = lj
                acc = oj
            else:
                alpha = jnp.exp2((m - m_new) * c)
                l = l * alpha + lj
                acc = acc * alpha + oj
            m = m_new
        s0_scr[...] = _qk(sb[s, o_q:o_q + M, :], sb[s, o_k0:o_k0 + C, :])
        lf = jnp.sum(l, axis=-1, keepdims=True)
        ob[g] = (acc / lf).astype(ob.dtype)
        pltpu.make_async_copy(ob.at[g], o_hbm.at[g], sem_out).start()
        return carry

    jax.lax.fori_loop(0, kf, functools.partial(body, fine=True), 0)
    jax.lax.fori_loop(kf, N, functools.partial(body, fine=False), 0)
    pltpu.make_async_copy(ob, o_hbm, sem_out).wait()


@jax.jit
def pallas_standalone__gqa_softmax__near_ridge_kernel(
    q: jax.Array,
    k: jax.Array,
    v: jax.Array,
):
    B, Hq, Sq, D = q.shape
    Hkv, Sk = k.shape[1], k.shape[2]
    rep = Hq // Hkv
    N = B * Hkv
    M = rep * Sq
    C = 256
    q3 = q.reshape(N, M, D)
    k3 = k.reshape(N, Sk, D)
    v3 = v.reshape(N, Sk, D)
    out = pl.pallas_call(
        functools.partial(_attn_kernel, C=C, startpos=6, tpos=6, kf=4),
        in_specs=[pl.BlockSpec(memory_space=pl.ANY)] * 3,
        out_specs=pl.BlockSpec(memory_space=pl.ANY),
        out_shape=jax.ShapeDtypeStruct((N, M, D), q.dtype),
        scratch_shapes=[
            pltpu.VMEM((_NG, 2 * Sk + M, D), q.dtype),
            pltpu.VMEM((N, M, D), q.dtype),
            pltpu.VMEM((M, C), jnp.float32),
            pltpu.VMEM((D, C), q.dtype),
            pltpu.SemaphoreType.DMA((_NG,)),
            pltpu.SemaphoreType.DMA((_NG,)),
            pltpu.SemaphoreType.DMA((_NG,)),
            pltpu.SemaphoreType.DMA((2,)),
            pltpu.SemaphoreType.DMA(()),
        ],
        compiler_params=pltpu.CompilerParams(
            vmem_limit_bytes=64 * 1024 * 1024,
            disable_bounds_checks=True),
    )(q3, k3, v3)
    return out.reshape(B, Hq, Sq, D)
```
